```python
import jax
import jax.numpy as jnp

def _softmax(x, axis=-1):
    return jax.nn.softmax(x, axis=axis)
def _gelu(x):
    return jax.nn.gelu(x, approximate=True)
def _silu(x):
    return jax.nn.silu(x)
def _sigmoid(x):
    return jax.nn.sigmoid(x)
def _layernorm(x, axis=-1, eps=1e-5):
    m = jnp.mean(x, axis=axis, keepdims=True)
    v = jnp.var(x, axis=axis, keepdims=True)
    return (x - m) / jnp.sqrt(v + eps)
def _scatter_add(tgt, idx, src, axis=0):
    return tgt.at[idx].add(src)
def _segment_sum(src, seg, n):
    return jax.ops.segment_sum(src, seg, n)
class _Rng:
    def __init__(self, key):
        self._k = key
    def _next(self):
        self._k, sub = jax.random.split(self._k)
        return sub
    def normal(self, shape):
        return jax.random.normal(self._next(), shape, dtype=jnp.bfloat16)
    def randint(self, lo, hi, shape):
        return jax.random.randint(self._next(), shape, lo, hi, dtype=jnp.int32)
    def uniform(self, shape, lo=0.0, hi=1.0):
        return jax.random.uniform(self._next(), shape, jnp.bfloat16, lo, hi)
    def permutation(self, n):
        return jax.random.permutation(self._next(), n)


kernel_name = 'standalone__instancenorm__prompt'

def setup_inputs():
    _rng = _Rng(jax.random.key(int.from_bytes(__import__("os").urandom(4), "little")))
    _w = (lambda a: (lambda t: t.astype(jnp.bfloat16) if jnp.issubdtype(t.dtype, jnp.floating) else t)(jnp.asarray(a)))
    B, C, H, W = 2, 1024, 2048, 32
    return {
        "x": _w((lambda *s: _rng.normal(s) * 0.05)(B, C, H, W)),
        "g": _w((lambda *s: _rng.normal(s) * 0.05)(C) + 1.0),
        "b": _w((lambda *s: _rng.normal(s) * 0.05)(C)),
    }

def reference(x, g, b):
    mu = x.mean(axis=(-2, -1), keepdims=True)
    var = ((x - mu) * (x - mu)).mean(axis=(-2, -1), keepdims=True)
    xhat = (x - mu) / jnp.sqrt(var + 1e-5)
    return xhat * g.reshape(1, -1, 1, 1) + b.reshape(1, -1, 1, 1)
```

```python
import jax
import jax.numpy as jnp
from jax import lax
import jax.experimental.pallas as pl
import jax.experimental.pallas.tpu as pltpu

_EPS = 1e-5
_LANES = 128
_ROWS = 16

_RS, _WS = 16, 8
_COLS = 16
_PIECE = 4
_CHUNK = 43
_R_TAIL = 11
_LEAD = 2
_GROUP = 4


def _make_kernel(B, C, H, W):
    V = H * W // (_ROWS * _LANES)
    ncol = B * C // _RS
    nchunk = pl.cdiv(ncol, _CHUNK)
    quads = _RS // 4
    steps = (V // _PIECE) * quads
    inv_n = 1.0 / (H * W)
    groups = [range(s, s + _GROUP) for s in range(0, _WS, _GROUP)]

    def kernel(x_hbm, g_hbm, b_hbm, o_hbm, buf, gb, gt, bt, r_sem, w_sem, g_sem):
        def split(col):
            return lax.div(col, _COLS), lax.rem(col, _COLS)

        def r_start(c0, j, t):
            g, jj = split(c0 + j)
            p, s = (t // quads) * _PIECE, (t % quads) * 2
            for q in range(2):
                pltpu.make_async_copy(
                    x_hbm.at[g, pl.ds(2 * (s + q), 2), pl.ds(jj * V + p, _PIECE)],
                    buf.at[s + q, :, pl.ds(j * V + p, _PIECE)],
                    r_sem.at[t],
                ).start(priority=q)

        def r_wait(j, t):
            p, s = (t // quads) * _PIECE, (t % quads) * 2
            dst = buf.at[pl.ds(s, 2), :, pl.ds(j * V + p, _PIECE)]
            pltpu.make_async_copy(dst, dst, r_sem.at[t]).wait()

        def w_copy(c0, u, p, n):
            j, h = lax.div(u, 2), lax.rem(u, 2)
            g, jj = split(c0 + j)
            return pltpu.make_async_copy(
                buf.at[:, h, pl.ds(j * V + p, n)],
                o_hbm.at[g, :, pl.ds((h * _COLS + jj) * V + p, n)],
                w_sem.at[lax.rem(u, _LEAD)],
            )

        def w_start(c0, u):
            for p in range(0, V, _PIECE):
                w_copy(c0, u, p, _PIECE).start()

        def w_wait(c0, u):
            w_copy(c0, u, 0, V).wait()

        def total(acc):
            return jnp.sum(jnp.sum(acc, axis=1, keepdims=True), axis=0, keepdims=True)

        def normalise(c0, u, streams):
            j, h = lax.div(u, 2), lax.rem(u, 2)
            g, jj = split(c0 + j)

            def val(s, k):
                return buf[s, h, j * V + k].astype(jnp.float32)

            means = []
            for s in streams:
                acc = val(s, 0)
                for k in range(1, V):
                    acc = acc + val(s, k)
                means.append(total(acc) * inv_n)
            affines = []
            for s, mu in zip(streams, means):
                acc = None
                for k in range(V):
                    d = val(s, k) - mu
                    acc = d * d if acc is None else acc + d * d
                ch = lax.rem((g * _RS + 2 * s + h) * _COLS + jj, C)
                scale = lax.rsqrt(total(acc) * inv_n + _EPS) * gt[pl.ds(ch, 1), :]
                affines.append((scale, bt[pl.ds(ch, 1), :]))
            for s, mu, (scale, shift) in zip(streams, means, affines):
                for k in range(V):
                    y = (val(s, k) - mu) * scale + shift
                    buf[s, h, j * V + k] = y.astype(buf.dtype)

        def loop(lo, hi, body):
            def wrapped(i, carry):
                body(i)
                return carry

            lax.fori_loop(lo, hi, wrapped, 0)

        zero = jnp.int32(0)
        for t in range(steps):
            r_start(zero, zero, t)

        copies = [
            pltpu.make_async_copy(src, gb.at[i], g_sem.at[i])
            for i, src in enumerate((g_hbm, b_hbm))
        ]
        for copy in copies:
            copy.start()
        for i, dst in enumerate((gt, bt)):
            copies[i].wait()
            v = gb[i].astype(jnp.float32)
            for k in range(C // _LANES):
                dst[pl.ds(k * _LANES, _LANES), :] = jnp.broadcast_to(
                    v[k : k + 1, :], (_LANES, _LANES)
                ).T

        def chunk(c):
            c0 = c * _CHUNK
            m = jnp.minimum(_CHUNK, ncol - c0)

            def read_column(j, work=()):
                every = steps // max(len(work), 1)
                for t in range(steps):
                    r_wait(j, t)
                    r_start(c0, j + 1, t)
                    if work and t % every == every - 1:
                        normalise(*work[t // every])

            first = pl.cdiv(_LEAD, 2)
            loop(0, first, read_column)
            loop(
                first,
                first + _LEAD,
                lambda j: read_column(j, [(c0, j - first, ss) for ss in groups]),
            )
            loop(first + _LEAD, m - 1, read_column)
            for t in range(steps):
                if steps - t == _R_TAIL:
                    for u in range(_LEAD):
                        w_start(c0, jnp.int32(u))
                r_wait(m - 1, t)

            def write_unit(u):
                for ss in groups:
                    normalise(c0, u + _LEAD, ss)
                w_wait(c0, u)
                w_start(c0, u + _LEAD)

            loop(0, 2 * m - _LEAD, write_unit)
            for i in range(_LEAD):
                w_wait(c0, 2 * m - _LEAD + i)

            @pl.when(c + 1 < nchunk)
            def _():
                for t in range(steps):
                    r_start(c0 + _CHUNK, zero, t)

        loop(0, nchunk, chunk)

    scratch = [
        pltpu.VMEM((_WS, 2, _CHUNK * V, _ROWS, _LANES), jnp.bfloat16),
        pltpu.VMEM((2, C // _LANES, _LANES), jnp.bfloat16),
        pltpu.VMEM((C, _LANES), jnp.float32),
        pltpu.VMEM((C, _LANES), jnp.float32),
        pltpu.SemaphoreType.DMA((steps,)),
        pltpu.SemaphoreType.DMA((_LEAD,)),
        pltpu.SemaphoreType.DMA((2,)),
    ]
    return kernel, scratch


@jax.jit
def pallas_standalone__instancenorm__prompt_kernel(
    x: jax.Array,
    g: jax.Array,
    b: jax.Array,
):
    B, C, H, W = x.shape
    kernel, scratch = _make_kernel(B, C, H, W)
    N = B * C
    V = H * W // (_ROWS * _LANES)
    G = N // (_RS * _COLS)
    xt = jnp.transpose(x, (0, 1, 3, 2)).reshape(N, W // 8, 8, H // _LANES, _LANES)
    xt = jnp.transpose(xt, (0, 1, 3, 2, 4)).reshape(G, _RS, _COLS * V, _ROWS, _LANES)
    y = pl.pallas_call(
        kernel,
        in_specs=[pl.BlockSpec(memory_space=pl.ANY)] * 3,
        out_specs=pl.BlockSpec(memory_space=pl.ANY),
        out_shape=jax.ShapeDtypeStruct((G, _WS, 2 * _COLS * V, _ROWS, _LANES), x.dtype),
        scratch_shapes=scratch,
        compiler_params=pltpu.CompilerParams(vmem_limit_bytes=110 * 1024 * 1024),
    )(xt, g.reshape(C // _LANES, _LANES), b.reshape(C // _LANES, _LANES))
    y = jnp.transpose(y.reshape(N, W // 8, H // _LANES, 8, _LANES), (0, 1, 3, 2, 4))
    return jnp.transpose(y.reshape(B, C, W, H), (0, 1, 3, 2))
```

```python
import jax
import jax.numpy as jnp
from jax import lax
import jax.experimental.pallas as pl
import jax.experimental.pallas.tpu as pltpu

_EPS = 1e-5
_LANES = 128
_ROWS = 16

_STREAMS = 8
_COLS = 8
_PIECE = 4
_GROUPS = 6
_STEPS = 4
_R_ROWS = 8
_R_PACE = 10
_R_TAIL = 7
_LEAD = 2
_TOGETHER = 4
_SLICE_ROWS = 3


def _div(a, n):
    if n & (n - 1) == 0:
        return lax.shift_right_logical(a, n.bit_length() - 1)
    return lax.div(a, n)


def _rem(a, n):
    return a & (n - 1) if n & (n - 1) == 0 else lax.rem(a, n)


def _loop(lo, hi, body):
    def wrapped(i, carry):
        body(i)
        return carry

    lax.fori_loop(lo, hi, wrapped, 0)


def _total(acc):
    return jnp.sum(jnp.sum(acc, axis=0, keepdims=True), axis=1, keepdims=True)


def _make_kernel(B, C, H, W):
    V = H * W // (_ROWS * _LANES)
    ngroup = B * C // (2 * _STREAMS * _COLS)
    nchunk = pl.cdiv(ngroup, _GROUPS)
    NP = V // _PIECE
    rpg = NP * _COLS
    inv_n = 1.0 / (H * W)

    def kernel(x_hbm, g_hbm, b_hbm, o_hbm, buf, gb, gt, bt, w_sem):
        def w_copy(g0, u, lo, hi, slot):
            blk = _div(u, _COLS)
            cols = pl.ds(_rem(u, _COLS) * V + lo * _PIECE, (hi - lo) * _PIECE)
            return pltpu.make_async_copy(
                buf.at[blk, :, :, :, cols],
                o_hbm.at[2 * g0 + blk, :, :, :, cols],
                w_sem.at[slot],
            )

        def w_start(g0, u, lo, hi, slot):
            for p in range(lo, hi):
                w_copy(g0, u, p, p + 1, slot).start()

        def normalise(g0, u, s):
            blk, col = _div(u, _COLS), _rem(u, _COLS)
            ref = buf.at[blk, _div(s, 4), _rem(_div(s, 2), 2), _rem(s, 2), pl.ds(col * V, V)]

            def val(k):
                return ref[k].astype(jnp.float32)

            acc = None
            for k in range(V):
                acc = val(k) if acc is None else acc + val(k)
                if k == V // 2 - 1:
                    yield
            mean = _total(acc)
            yield
            yield
            mean = mean * inv_n
            acc = None
            for k in range(V):
                d = val(k) - mean
                acc = d * d if acc is None else acc + d * d
                if k in (V // 3, 2 * V // 3):
                    yield
            var = _total(acc)
            yield
            yield
            ch = _rem(((2 * g0 + blk) * _STREAMS + s) * _COLS + col, C)
            scale = lax.rsqrt(var * inv_n + _EPS) * gt[pl.ds(ch, 1), :]
            shift = bt[pl.ds(ch, 1), :]
            yield
            for k in range(V):
                ref[k] = ((val(k) - mean) * scale + shift).astype(ref.dtype)
                if k % (V // 4) == V // 4 - 1 and k < V - 1:
                    yield

        def load_affine(sem):
            copies = [
                pltpu.make_async_copy(src, gb.at[i], sem.at[i])
                for i, src in enumerate((g_hbm, b_hbm))
            ]
            for copy in copies:
                copy.start()
            for i, dst in enumerate((gt, bt)):
                copies[i].wait()
                v = gb[i].astype(jnp.float32)
                for k in range(C // _LANES):
                    dst[pl.ds(k * _LANES, _LANES), :] = jnp.broadcast_to(
                        v[k : k + 1, :], (_LANES, _LANES)
                    ).T

        def wait_last_write(g0, u):
            w_copy(g0, u, NP - 1, NP, _LEAD).wait()

        def read_phase(c, g0, nrow, r_sem):
            def locate(i, t):
                i, a = i + t // _STEPS, t % _STEPS
                cols = pl.ds(_rem(i, rpg) * _PIECE, _PIECE)
                sem = r_sem.at[_rem(i, _R_ROWS) * _STEPS + a]
                return 2 * _div(i, rpg) + a // 2, a % 2, cols, sem

            def start(i, t, priority):
                blk, a, cols, sem = locate(i, t)
                pltpu.make_async_copy(
                    x_hbm.at[2 * g0 + blk, a, :, 1 - priority, cols],
                    buf.at[blk, a, :, 1 - priority, cols],
                    sem,
                ).start(priority=priority)

            def wait(i, t):
                blk, a, cols, sem = locate(i, t)
                dst = buf.at[blk, a, :, :, cols]
                pltpu.make_async_copy(dst, dst, sem).wait()

            win = _STEPS * _R_ROWS
            zero = jnp.int32(0)
            for t in range(win):
                start(zero, t, 1)
                if t < _R_PACE:
                    start(zero, t, 0)

            @pl.when(c > 0)
            def _():
                prev = _div((c - 1) * ngroup, nchunk)
                wait_last_write(prev, 2 * (g0 - prev) * _COLS - 1)

            @pl.when(c == 0)
            def _():
                pl.run_scoped(load_affine, pltpu.SemaphoreType.DMA((2,)))

            def row(i, work=None):
                for a in range(_STEPS):
                    wait(i, a)
                    start(i, a + _R_PACE, 0)
                    start(i, a + win, 1)
                    if work is not None:
                        next(work, None)

            def rows_and_instance(k):
                work = normalise(g0, _div(k, _STREAMS), _rem(k, _STREAMS))
                for r in range(_SLICE_ROWS):
                    row(NP + _SLICE_ROWS * k + r, work)
                for _ in work:
                    pass

            _loop(0, NP, row)
            _loop(0, _STREAMS * _LEAD, rows_and_instance)
            _loop(NP + _SLICE_ROWS * _STREAMS * _LEAD, nrow - _R_ROWS, row)
            for t in range(win):
                if win - t == _R_TAIL:
                    w_start(g0, zero, 0, NP, 0)
                wait(nrow - _R_ROWS, t)
                if t + _R_PACE < win:
                    start(nrow - _R_ROWS, t + _R_PACE, 0)
            for u in range(1, _LEAD):
                w_start(g0, jnp.int32(u), 0, NP, u)

        def write_phase(g0, nunit):
            def unit(u):
                def some(k):
                    work = [
                        normalise(g0, u + _LEAD, k * _TOGETHER + s)
                        for s in range(_TOGETHER)
                    ]
                    while work:
                        work = [w for w in work if next(w, w) is not w]

                _loop(0, _STREAMS // _TOGETHER, some)
                slot = _rem(u, _LEAD)
                w_copy(g0, u, 0, NP, slot).wait()
                w_start(g0, u + _LEAD, 0, NP - 1, slot)
                slot = jnp.where(u + _LEAD == nunit - 1, _LEAD, slot)
                w_start(g0, u + _LEAD, NP - 1, NP, slot)

            _loop(0, nunit - _LEAD, unit)
            for i in range(_LEAD):
                u = nunit - _LEAD + i
                w_copy(g0, u, 0, NP - (i == _LEAD - 1), _rem(u, _LEAD)).wait()

        def chunk(c):
            g0 = _div(c * ngroup, nchunk)
            ng = _div((c + 1) * ngroup, nchunk) - g0
            pl.run_scoped(
                lambda r_sem: read_phase(c, g0, ng * rpg, r_sem),
                pltpu.SemaphoreType.DMA((_STEPS * _R_ROWS,)),
            )
            write_phase(g0, 2 * ng * _COLS)

        _loop(0, nchunk, chunk)
        last = (nchunk - 1) * ngroup // nchunk
        wait_last_write(jnp.int32(last), jnp.int32(2 * (ngroup - last) * _COLS - 1))

    scratch = [
        pltpu.VMEM((2 * _GROUPS, 2, 2, 2, _COLS * V, _ROWS, _LANES), jnp.bfloat16),
        pltpu.VMEM((2, C // _LANES, _LANES), jnp.bfloat16),
        pltpu.VMEM((C, _LANES), jnp.float32),
        pltpu.VMEM((C, _LANES), jnp.float32),
        pltpu.SemaphoreType.DMA((_LEAD + 1,)),
    ]
    return kernel, scratch


@jax.jit
def pallas_standalone__instancenorm__prompt_kernel(
    x: jax.Array,
    g: jax.Array,
    b: jax.Array,
):
    B, C, H, W = x.shape
    kernel, scratch = _make_kernel(B, C, H, W)
    N = B * C
    V = H * W // (_ROWS * _LANES)
    shape = (N // (_STREAMS * _COLS), 2, 2, 2, _COLS * V, _ROWS, _LANES)
    xt = jnp.transpose(x, (0, 1, 3, 2)).reshape(N, W // 8, 8, H // _LANES, _LANES)
    xt = jnp.transpose(xt, (0, 1, 3, 2, 4)).reshape(shape)
    y = pl.pallas_call(
        kernel,
        in_specs=[pl.BlockSpec(memory_space=pl.ANY)] * 3,
        out_specs=pl.BlockSpec(memory_space=pl.ANY),
        out_shape=jax.ShapeDtypeStruct(shape, x.dtype),
        scratch_shapes=scratch,
        compiler_params=pltpu.CompilerParams(vmem_limit_bytes=112 * 1024 * 1024),
    )(xt, g.reshape(C // _LANES, _LANES), b.reshape(C // _LANES, _LANES))
    y = jnp.transpose(y.reshape(N, W // 8, H // _LANES, 8, _LANES), (0, 1, 3, 2, 4))
    return jnp.transpose(y.reshape(B, C, W, H), (0, 1, 3, 2))
```

```python
import jax
import jax.numpy as jnp
from jax import lax
import jax.experimental.pallas as pl
import jax.experimental.pallas.tpu as pltpu

_EPS = 1e-5
_LANES = 128
_ROWS = 16

_STREAMS = 8
_COLS = 8
_PIECE = 4
_GROUPS = 8
_STEPS = 4
_R_ROWS = 4
_R_PACE = 9
_R_TAIL = 6
_LEAD = 2
_UNROLL = 8
_SLICE_ROWS = 3


def _div(a, n):
    assert n & (n - 1) == 0
    return lax.shift_right_logical(a, n.bit_length() - 1)


def _rem(a, n):
    assert n & (n - 1) == 0
    return a & (n - 1)


def _loop(lo, hi, body):
    def wrapped(i, carry):
        body(i)
        return carry

    lax.fori_loop(lo, hi, wrapped, 0)


def _total(acc):
    return jnp.sum(jnp.sum(acc, axis=0, keepdims=True), axis=1, keepdims=True)


def _fold(v):
    return v[: _ROWS // 2] + v[_ROWS // 2 :]


def _pick(table, ch):
    pos = lax.broadcasted_iota(jnp.int32, table.shape, 0) * _LANES
    pos = pos + lax.broadcasted_iota(jnp.int32, table.shape, 1)
    return _total(jnp.where(pos == ch, table, 0.0))


def _make_kernel(B, C, H, W):
    V = H * W // (_ROWS * _LANES)
    NP = V // _PIECE
    nchunk = B * C // (_GROUPS * 2 * _STREAMS * _COLS)
    nunit = _GROUPS * 2 * _COLS
    nrow = _GROUPS * _COLS * NP
    width = 2 * _STREAMS // _STEPS
    inv_n = 1.0 / (H * W)

    def kernel(x_hbm, g_hbm, b_hbm, o_hbm, buf, w_sem):
        def locate(u):
            blk = _div(u, _COLS)
            return _div(blk, 2), _rem(blk, 2) * _STREAMS, _rem(u, _COLS) * V

        def w_copy(c, u, lo, hi):
            grp, s0, k0 = locate(u)
            ss = pl.ds(s0, _STREAMS)
            kk = pl.ds(k0 + lo * _PIECE, (hi - lo) * _PIECE)
            return pltpu.make_async_copy(
                buf.at[grp, ss, kk],
                o_hbm.at[c * _GROUPS + grp, ss, kk],
                w_sem.at[_rem(u, _LEAD)],
            )

        def w_start(c, u):
            for p in range(NP):
                w_copy(c, u, p, p + 1).start()

        def w_wait(c, u):
            w_copy(c, u, 0, NP).wait()

        def instance(c, u, s):
            grp, s0, k0 = locate(u)
            n = ((c * _GROUPS + grp) * 2 * _STREAMS + s0 + s) * _COLS + _rem(u, _COLS)
            return buf.at[grp, s0 + s, pl.ds(k0, V)], _rem(n, C)

        def normalise_sliced(affine, c, u, s):
            ref, ch = instance(c, u, s)
            acc = 0.0
            for k in range(V):
                acc = acc + ref[k].astype(jnp.float32)
                if k == V // 2 - 1:
                    yield
            mean = _total(acc)
            yield
            gain, shift = (_pick(table, ch) for table in affine)
            yield
            mean = mean * inv_n
            acc = 0.0
            for k in range(V):
                d = ref[k].astype(jnp.float32) - mean
                acc = acc + d * d
                if k in (V // 3, 2 * V // 3):
                    yield
            var = _total(acc)
            yield
            yield
            scale = lax.rsqrt(var * inv_n + _EPS) * gain
            yield
            for k in range(V):
                y = (ref[k].astype(jnp.float32) - mean) * scale + shift
                ref[k] = y.astype(ref.dtype)
                if k % (V // 4) == V // 4 - 1 and k < V - 1:
                    yield

        def normalise_unit(affine, c, u):
            refs, chs = zip(*(instance(c, u, s) for s in range(_STREAMS)))

            def totals(term):
                def body(i, accs):
                    for k in range(_UNROLL):
                        accs = [
                            acc + _fold(term(s, ref[i * _UNROLL + k].astype(jnp.float32)))
                            for s, (acc, ref) in enumerate(zip(accs, refs))
                        ]
                    return accs

                init = [jnp.zeros((_ROWS // 2, _LANES), jnp.float32)] * _STREAMS
                return [_total(acc) for acc in lax.fori_loop(0, V // _UNROLL, body, init)]

            means = [t * inv_n for t in totals(lambda s, v: v)]
            squares = totals(lambda s, v: (v - means[s]) * (v - means[s]))
            scales = [
                lax.rsqrt(t * inv_n + _EPS) * _pick(affine[0], ch)
                for t, ch in zip(squares, chs)
            ]
            shifts = [_pick(affine[1], ch) for ch in chs]

            def apply(i):
                for k in range(_UNROLL):
                    for ref, mean, scale, shift in zip(refs, means, scales, shifts):
                        v = ref[i * _UNROLL + k].astype(jnp.float32)
                        ref[i * _UNROLL + k] = ((v - mean) * scale + shift).astype(ref.dtype)

            _loop(0, V // _UNROLL, apply)

        def load_affine(sem):
            last = buf.at[_GROUPS - 1, 2 * _STREAMS - 1]
            dsts = [last.at[_COLS * V - 1 - i, pl.ds(0, C // _LANES)] for i in range(2)]
            copies = [
                pltpu.make_async_copy(src, dst, sem.at[i])
                for i, (src, dst) in enumerate(zip((g_hbm, b_hbm), dsts))
            ]
            for copy in copies:
                copy.start()
            for copy in copies:
                copy.wait()
            return tuple(dst[...].astype(jnp.float32) for dst in dsts)

        def read_phase(c, affine, r_sem):
            def step(i, t):
                i, a = i + t // _STEPS, t % _STEPS
                kk = pl.ds(_rem(i, _COLS * NP) * _PIECE, _PIECE)
                sem = r_sem.at[_rem(i, _R_ROWS) * _STEPS + a]
                return _div(i, _COLS * NP), a * width, kk, sem

            def start(i, t, priority):
                grp, s0, kk, sem = step(i, t)
                ss = pl.ds(s0, width - 1) if priority else pl.ds(s0 + width - 1, 1)
                pltpu.make_async_copy(
                    x_hbm.at[c * _GROUPS + grp, ss, kk], buf.at[grp, ss, kk], sem
                ).start(priority=priority)

            def wait(i, t):
                grp, s0, kk, sem = step(i, t)
                dst = buf.at[grp, pl.ds(s0, width), kk]
                pltpu.make_async_copy(dst, dst, sem).wait()

            win = _STEPS * _R_ROWS
            zero = jnp.int32(0)
            for t in range(win):
                start(zero, t, 1)
                if t < _R_PACE:
                    start(zero, t, 0)

            affine = lax.cond(
                c == 0,
                lambda: pl.run_scoped(load_affine, pltpu.SemaphoreType.DMA((2,))),
                lambda: affine,
            )

            def row(i, work=None):
                for a in range(_STEPS):
                    wait(i, a)
                    start(i, a + _R_PACE, 0)
                    start(i, a + win, 1)
                    if work is not None:
                        next(work, None)

            def rows_and_instance(k):
                work = normalise_sliced(affine, c, _div(k, _STREAMS), _rem(k, _STREAMS))
                for r in range(_SLICE_ROWS):
                    row(NP + _SLICE_ROWS * k + r, work)
                for _ in work:
                    pass

            _loop(0, NP, row)
            _loop(0, _STREAMS * _LEAD, rows_and_instance)
            _loop(NP + _SLICE_ROWS * _STREAMS * _LEAD, nrow - _R_ROWS, row)
            tail = jnp.int32(nrow - _R_ROWS)
            for t in range(win):
                if win - t == _R_TAIL:
                    w_start(c, zero)
                wait(tail, t)
                if t + _R_PACE < win:
                    start(tail, t + _R_PACE, 0)
            for u in range(1, _LEAD):
                w_start(c, jnp.int32(u))
            return affine

        def chunk(c, affine):
            affine = pl.run_scoped(
                lambda r_sem: read_phase(c, affine, r_sem),
                pltpu.SemaphoreType.DMA((_STEPS * _R_ROWS,)),
            )

            def write_unit(u):
                normalise_unit(affine, c, u + _LEAD)
                w_wait(c, u)
                w_start(c, u + _LEAD)

            _loop(0, nunit - _LEAD, write_unit)
            for u in range(nunit - _LEAD, nunit):
                w_wait(c, jnp.int32(u))
            return affine

        blank = jnp.zeros((C // _LANES, _LANES), jnp.float32)
        lax.fori_loop(0, nchunk, chunk, (blank, blank))

    scratch = [
        pltpu.VMEM((_GROUPS, 2 * _STREAMS, _COLS * V, _ROWS, _LANES), jnp.bfloat16),
        pltpu.SemaphoreType.DMA((_LEAD,)),
    ]
    return kernel, scratch


@jax.jit
def pallas_standalone__instancenorm__prompt_kernel(
    x: jax.Array,
    g: jax.Array,
    b: jax.Array,
):
    B, C, H, W = x.shape
    kernel, scratch = _make_kernel(B, C, H, W)
    N = B * C
    V = H * W // (_ROWS * _LANES)
    shape = (N // (2 * _STREAMS * _COLS), 2 * _STREAMS, _COLS * V, _ROWS, _LANES)
    xt = jnp.transpose(x, (0, 1, 3, 2)).reshape(N, W // 8, 8, H // _LANES, _LANES)
    xt = jnp.transpose(xt, (0, 1, 3, 2, 4)).reshape(shape)
    y = pl.pallas_call(
        kernel,
        in_specs=[pl.BlockSpec(memory_space=pl.ANY)] * 3,
        out_specs=pl.BlockSpec(memory_space=pl.ANY),
        out_shape=jax.ShapeDtypeStruct(shape, x.dtype),
        scratch_shapes=scratch,
        compiler_params=pltpu.CompilerParams(vmem_limit_bytes=128 * 1024 * 1024),
    )(xt, g.reshape(C // _LANES, _LANES), b.reshape(C // _LANES, _LANES))
    y = jnp.transpose(y.reshape(N, W // 8, H // _LANES, 8, _LANES), (0, 1, 3, 2, 4))
    return jnp.transpose(y.reshape(B, C, W, H), (0, 1, 3, 2))
```

```python
import jax
import jax.numpy as jnp
from jax import lax
import jax.experimental.pallas as pl
import jax.experimental.pallas.tpu as pltpu

_EPS = 1e-5
_LANES = 128
_ROWS = 16

_COLS = 8
_PIECE = 4
_HELD = 128

_R_BLOCK = 16
_R_STEPS = ((0, 4), (4, 4), (8, 4), (12, 4))
_R_ROWS = 4
_R_PACE = 9
_R_TAIL = 6

_W_SEGMENTS = ((0, 2, 8), (16, 16, 7))
_LEAD = 2

_UNROLL = 16
_SLICE_ROWS = 3


def _div(a, n):
    assert n & (n - 1) == 0
    return lax.shift_right_logical(a, n.bit_length() - 1)


def _rem(a, n):
    assert n & (n - 1) == 0
    return a & (n - 1)


def _loop(lo, hi, body):
    def wrapped(i, carry):
        body(i)
        return carry

    lax.fori_loop(lo, hi, wrapped, 0)


def _total(acc):
    return jnp.sum(jnp.sum(acc, axis=0, keepdims=True), axis=1, keepdims=True)


def _fold(v):
    return v[: _ROWS // 2] + v[_ROWS // 2 :]


def _pick(table, ch):
    pos = lax.broadcasted_iota(jnp.int32, table.shape, 0) * _LANES
    pos = pos + lax.broadcasted_iota(jnp.int32, table.shape, 1)
    return _total(jnp.where(pos == ch, table, 0.0))


def _make_kernel(B, C, H, W):
    V = H * W // (_ROWS * _LANES)
    NP = V // _PIECE
    nchunk = B * C // (_HELD * _COLS)
    nrow = _HELD // _R_BLOCK * _COLS * NP
    nstep = len(_R_STEPS)
    head = _W_SEGMENTS[0]
    inv_n = 1.0 / (H * W)

    def kernel(x_hbm, g_hbm, b_hbm, o_hbm, buf, w_sem):
        def first_stream(seg, u):
            return seg[0] + _div(u, _COLS) * seg[2]

        def w_copy(c, seg, u, lo, hi):
            s0 = first_stream(seg, u)
            kk = pl.ds(_rem(u, _COLS) * V + lo * _PIECE, (hi - lo) * _PIECE)
            return pltpu.make_async_copy(
                buf.at[pl.ds(s0, seg[2]), kk],
                o_hbm.at[pl.ds(c * _HELD + s0, seg[2]), kk],
                w_sem.at[_rem(u, _LEAD)],
            )

        def w_start(c, seg, u):
            for p in range(NP):
                w_copy(c, seg, u, p, p + 1).start()

        def w_wait(c, seg, u):
            w_copy(c, seg, u, 0, NP).wait()

        def instance(c, seg, u, s):
            s, col = first_stream(seg, u) + s, _rem(u, _COLS)
            return buf.at[s, pl.ds(col * V, V)], _rem((c * _HELD + s) * _COLS + col, C)

        def normalise_sliced(affine, c, u, s):
            ref, ch = instance(c, head, u, s)
            acc = 0.0
            for k in range(V):
                acc = acc + ref[k].astype(jnp.float32)
                if k == V // 2 - 1:
                    yield
            mean = _total(acc)
            yield
            gain, shift = (_pick(table, ch) for table in affine)
            yield
            mean = mean * inv_n
            acc = 0.0
            for k in range(V):
                d = ref[k].astype(jnp.float32) - mean
                acc = acc + d * d
                if k in (V // 3, 2 * V // 3):
                    yield
            var = _total(acc)
            yield
            yield
            scale = lax.rsqrt(var * inv_n + _EPS) * gain
            yield
            for k in range(V):
                y = (ref[k].astype(jnp.float32) - mean) * scale + shift
                ref[k] = y.astype(ref.dtype)
                if k % (V // 4) == V // 4 - 1 and k < V - 1:
                    yield

        def normalise_unit(affine, c, seg, u):
            refs, chs = zip(*(instance(c, seg, u, s) for s in range(seg[2])))

            def totals(term):
                def body(i, accs):
                    for k in range(_UNROLL):
                        accs = [
                            acc + _fold(term(s, ref[i * _UNROLL + k].astype(jnp.float32)))
                            for s, (acc, ref) in enumerate(zip(accs, refs))
                        ]
                    return accs

                init = [jnp.zeros((_ROWS // 2, _LANES), jnp.float32)] * len(refs)
                return [_total(acc) for acc in lax.fori_loop(0, V // _UNROLL, body, init)]

            means = [t * inv_n for t in totals(lambda s, v: v)]
            squares = totals(lambda s, v: (v - means[s]) * (v - means[s]))
            scales = [
                lax.rsqrt(t * inv_n + _EPS) * _pick(affine[0], ch)
                for t, ch in zip(squares, chs)
            ]
            shifts = [_pick(affine[1], ch) for ch in chs]

            def apply(i):
                for k in range(_UNROLL):
                    for ref, mean, scale, shift in zip(refs, means, scales, shifts):
                        v = ref[i * _UNROLL + k].astype(jnp.float32)
                        ref[i * _UNROLL + k] = ((v - mean) * scale + shift).astype(ref.dtype)

            _loop(0, V // _UNROLL, apply)

        def load_affine(sem):
            dsts = [
                buf.at[_HELD - 1, _COLS * V - 1 - i, pl.ds(0, C // _LANES)]
                for i in range(2)
            ]
            copies = [
                pltpu.make_async_copy(src, dst, sem.at[i])
                for i, (src, dst) in enumerate(zip((g_hbm, b_hbm), dsts))
            ]
            for copy in copies:
                copy.start()
            for copy in copies:
                copy.wait()
            return tuple(dst[...].astype(jnp.float32) for dst in dsts)

        def read_phase(c, affine, r_sem):
            def step(i, t):
                i, a = i + t // nstep, t % nstep
                s0, n = _R_STEPS[a]
                kk = pl.ds(_rem(i, _COLS * NP) * _PIECE, _PIECE)
                sem = r_sem.at[_rem(i, _R_ROWS) * nstep + a]
                return _div(i, _COLS * NP) * _R_BLOCK + s0, n, kk, sem

            def start(i, t, priority):
                s0, n, kk, sem = step(i, t)
                s0, n = (s0, n - 1) if priority else (s0 + n - 1, 1)
                pltpu.make_async_copy(
                    x_hbm.at[pl.ds(c * _HELD + s0, n), kk], buf.at[pl.ds(s0, n), kk], sem
                ).start(priority=priority)

            def wait(i, t):
                s0, n, kk, sem = step(i, t)
                dst = buf.at[pl.ds(s0, n), kk]
                pltpu.make_async_copy(dst, dst, sem).wait()

            win = nstep * _R_ROWS
            zero = jnp.int32(0)
            for t in range(win):
                start(zero, t, 1)
                if t < _R_PACE:
                    start(zero, t, 0)

            affine = lax.cond(
                c == 0,
                lambda: pl.run_scoped(load_affine, pltpu.SemaphoreType.DMA((2,))),
                lambda: affine,
            )

            def row(i, work=None):
                for a in range(nstep):
                    wait(i, a)
                    start(i, a + _R_PACE, 0)
                    start(i, a + win, 1)
                    if work is not None:
                        next(work, None)

            def rows_and_instance(k):
                work = normalise_sliced(affine, c, _div(k, head[2]), _rem(k, head[2]))
                for r in range(_SLICE_ROWS):
                    row(NP + _SLICE_ROWS * k + r, work)
                for _ in work:
                    pass

            _loop(0, NP, row)
            _loop(0, head[2] * _LEAD, rows_and_instance)
            _loop(NP + _SLICE_ROWS * head[2] * _LEAD, nrow - _R_ROWS, row)
            tail = jnp.int32(nrow - _R_ROWS)
            for t in range(win):
                if win - t == _R_TAIL:
                    w_start(c, head, zero)
                wait(tail, t)
                if t + _R_PACE < win:
                    start(tail, t + _R_PACE, 0)
            for u in range(1, _LEAD):
                w_start(c, head, jnp.int32(u))
            return affine

        def write_phase(c, affine):
            for prev, seg in zip((None,) + _W_SEGMENTS, _W_SEGMENTS):

                def unit(u, prev=prev, seg=seg):
                    normalise_unit(affine, c, seg, u)
                    if prev is None:
                        w_wait(c, seg, u - _LEAD)
                    else:
                        done = prev[1] * _COLS + u - _LEAD
                        pl.when(u < _LEAD)(lambda: w_wait(c, prev, done))
                        pl.when(u >= _LEAD)(lambda: w_wait(c, seg, u - _LEAD))
                    w_start(c, seg, u)

                _loop(_LEAD if prev is None else 0, seg[1] * _COLS, unit)
            last = _W_SEGMENTS[-1]
            for u in range(last[1] * _COLS - _LEAD, last[1] * _COLS):
                w_wait(c, last, jnp.int32(u))

        def chunk(c, affine):
            affine = pl.run_scoped(
                lambda r_sem: read_phase(c, affine, r_sem),
                pltpu.SemaphoreType.DMA((nstep * _R_ROWS,)),
            )
            write_phase(c, affine)
            return affine

        blank = jnp.zeros((C // _LANES, _LANES), jnp.float32)
        lax.fori_loop(0, nchunk, chunk, (blank, blank))

    scratch = [
        pltpu.VMEM((_HELD, _COLS * V, _ROWS, _LANES), jnp.bfloat16),
        pltpu.SemaphoreType.DMA((_LEAD,)),
    ]
    return kernel, scratch


@jax.jit
def pallas_standalone__instancenorm__prompt_kernel(
    x: jax.Array,
    g: jax.Array,
    b: jax.Array,
):
    B, C, H, W = x.shape
    kernel, scratch = _make_kernel(B, C, H, W)
    N = B * C
    shape = (N // _COLS, _COLS * H * W // (_ROWS * _LANES), _ROWS, _LANES)
    xt = jnp.transpose(x, (0, 1, 3, 2)).reshape(N, W // 8, 8, H // _LANES, _LANES)
    xt = jnp.transpose(xt, (0, 1, 3, 2, 4)).reshape(shape)
    y = pl.pallas_call(
        kernel,
        in_specs=[pl.BlockSpec(memory_space=pl.ANY)] * 3,
        out_specs=pl.BlockSpec(memory_space=pl.ANY),
        out_shape=jax.ShapeDtypeStruct(shape, x.dtype),
        scratch_shapes=scratch,
        compiler_params=pltpu.CompilerParams(vmem_limit_bytes=128 * 1024 * 1024),
    )(xt, g.reshape(C // _LANES, _LANES), b.reshape(C // _LANES, _LANES))
    y = jnp.transpose(y.reshape(N, W // 8, H // _LANES, 8, _LANES), (0, 1, 3, 2, 4))
    return jnp.transpose(y.reshape(B, C, W, H), (0, 1, 3, 2))
```
